```python
import os as _os
_os.environ.setdefault("JAX_PLATFORMS", "cpu")
import jax
import jax.numpy as jnp

def _softmax(x, axis=-1):
    return jax.nn.softmax(x, axis=axis)
def _gelu(x):
    return jax.nn.gelu(x, approximate=True)
def _silu(x):
    return jax.nn.silu(x)
def _sigmoid(x):
    return jax.nn.sigmoid(x)
def _layernorm(x, axis=-1, eps=1e-5):
    m = jnp.mean(x, axis=axis, keepdims=True)
    v = jnp.var(x, axis=axis, keepdims=True)
    return (x - m) / jnp.sqrt(v + eps)
def _scatter_add(tgt, idx, src, axis=0):
    return tgt.at[idx].add(src)
def _segment_sum(src, seg, n):
    return jax.ops.segment_sum(src, seg, n)
class _Rng:
    def __init__(self, key):
        self._k = key
    def _next(self):
        self._k, sub = jax.random.split(self._k)
        return sub
    def normal(self, shape):
        return jax.random.normal(self._next(), shape, dtype=jnp.bfloat16)
    def randint(self, lo, hi, shape):
        return jax.random.randint(self._next(), shape, lo, hi, dtype=jnp.int32)
    def uniform(self, shape, lo=0.0, hi=1.0):
        return jax.random.uniform(self._next(), shape, jnp.bfloat16, lo, hi)
    def permutation(self, n):
        return jax.random.permutation(self._next(), n)


kernel_name = 'sequential_preLN__sliding_local_dilated__dense_activation_relu__prompt'

def setup_inputs():
    _rng = _Rng(jax.random.key(int.from_bytes(__import__("os").urandom(4), "little")))
    _w = (lambda a: (lambda t: t.astype(jnp.bfloat16) if jnp.issubdtype(t.dtype, jnp.floating) else t)(jnp.asarray(a)))
    def _A_setup():
        B, S, D = 1, 2048, 1024
        return {
            "x": _w((lambda *s: _rng.normal(s) * 0.05)(B, S, D)),
            "wqkv": _w((lambda *s: _rng.normal(s) * 0.05)(D, 3 * D)),
            "wo": _w((lambda *s: _rng.normal(s) * 0.05)(D, D)),
        }
    _A_in = _A_setup()

    def _B_setup():
        B, S, D, Dff = 1, 2048, 1024, 3584
        return {
            "x": _w((lambda *s: _rng.normal(s) * 0.05)(B, S, D)),
            "w1": _w((lambda *s: _rng.normal(s) * 0.05)(D, Dff)),
            "w2": _w((lambda *s: _rng.normal(s) * 0.05)(Dff, D)),
        }
    _B_in = _B_setup()

    return {
        "A_x": _A_in["x"],
        "A_wqkv": _A_in["wqkv"],
        "A_wo": _A_in["wo"],
        "B_x": _B_in["x"],
        "B_w1": _B_in["w1"],
        "B_w2": _B_in["w2"],
    }

def reference(A_x, A_wqkv, A_wo, B_x, B_w1, B_w2):
    def _A_ref(x, wqkv, wo):
        B, S, D = x.shape
        H = 32; Dh = D // H
        W, dil = 8, 2
        qkv = (lambda x, *d: x.transpose(*d))((x @ wqkv).reshape(B, S, 3, H, Dh), 2, 0, 3, 1, 4)
        q, k, v = qkv[0], qkv[1], qkv[2]
        scale = Dh ** -0.5
        pos = jnp.arange(S)
        off = jnp.arange(W) * dil
        idx = pos[:, None] - off[None, :]
        mask = idx >= 0
        idx_c = jnp.where(mask, idx, 0).reshape(-1)
        kg = k[:, :, idx_c, :].reshape(B, H, S, W, Dh)
        vg = v[:, :, idx_c, :].reshape(B, H, S, W, Dh)
        logits = jnp.einsum("bhsd,bhswd->bhsw", q, kg) * scale
        logits = jnp.where(mask[None, None, :, :], logits, -1e9)
        attn = _softmax(logits, axis=-1)
        o = jnp.einsum("bhsw,bhswd->bhsd", attn, vg)
        return (lambda x, *d: x.transpose(*d))(o, 0, 2, 1, 3).reshape(B, S, D) @ wo

    def _B_ref(x, w1, w2):
        h = jnp.einsum("bsd,df->bsf", x, w1)
        zero = jnp.zeros_like(h)
        h = jnp.maximum(h, zero)
        return jnp.einsum("bsf,fd->bsd", h, w2)

    x = A_x
    h = x + _A_ref(_layernorm(x, axis=-1), A_wqkv, A_wo)
    h2 = h + _B_ref(_layernorm(h, axis=-1), B_w1, B_w2)
    return h2
```

```python
import numpy as np
import jax, jax.numpy as jnp
from jax.experimental import pallas as pl
from jax.experimental.pallas import tpu as pltpu

T = 256
R = 16
HALO = 16
VMEM_MB = 100
ROT3 = False

H, DH, W, DIL = 32, 32, 8, 2
NT = (((1,), (1,)), ((), ()))


def _ln(x):
    m = jnp.mean(x, axis=-1, keepdims=True)
    c = x - m
    v = jnp.mean(c * c, axis=-1, keepdims=True)
    return c * jax.lax.rsqrt(v + 1e-5)


def _scatter_pairs(src_u32, j, e_ref, o_ref):
    for h_lo in range(4):
        h = 4 * j + h_lo
        dst = o_ref if h % 2 else e_ref
        for a in range(8):
            dst[a, pl.ds((h // 2) * 17, 16), :] = src_u32[16 * h_lo:16 * h_lo + 16, 128 * a:128 * a + 128]


def _gather_pairs(e_ref, o_ref, dst_ref, base):
    for dp in range(16):
        for a in range(8):
            A = e_ref[a, pl.ds(dp, 16, stride=17), :]
            B = o_ref[a, pl.ds(dp, 16, stride=17), :]
            lo = (A & jnp.uint32(0xFFFF)) | (B << 16)
            hi = (A >> 16) | (B & jnp.uint32(0xFFFF0000))
            dst_ref[pl.ds(base + 32 * dp, 16), 128 * a:128 * a + 128] = lo
            dst_ref[pl.ds(base + 32 * dp + 16, 16), 128 * a:128 * a + 128] = hi


@jax.jit
def pallas_sequential_preLN__sliding_local_dilated__dense_activation_relu__prompt_kernel(
    A_x: jax.Array,
    A_wqkv: jax.Array,
    A_wo: jax.Array,
    B_x: jax.Array,
    B_w1: jax.Array,
    B_w2: jax.Array,
):
    _, S, D = A_x.shape
    x2 = A_x.reshape(S, D)
    scale = DH ** -0.5

    def kern(x_ref, wqkv_ref, wo_ref, w1_ref, w2_ref, out_ref,
             wt_ref, wop_ref, e_ref, o_ref, q_scr, k_scr, v_scr, a_scr):
        step = pl.program_id(0)

        @pl.when(step == 0)
        def _():
            for part in range(3):
                for j in range(8):
                    c0 = part * D + 128 * j
                    wt = wqkv_ref[:, c0:c0 + 128].T
                    _scatter_pairs(pltpu.bitcast(wt, jnp.uint32), j, e_ref, o_ref)
                _gather_pairs(e_ref, o_ref, wt_ref, part * 512)
            for j in range(8):
                _scatter_pairs(pltpu.bitcast(wo_ref[128 * j:128 * j + 128, :], jnp.uint32), j, e_ref, o_ref)
            _gather_pairs(e_ref, o_ref, wop_ref, 0)
            k_scr[:, 0:HALO, :] = jnp.zeros((8, HALO, 128), jnp.float32)
            v_scr[:, 0:HALO, :] = jnp.zeros((8, HALO, 128), jnp.float32)

        @pl.when(step > 0)
        def _():
            k_scr[:, 0:HALO, :] = k_scr[:, T:T + HALO, :]
            v_scr[:, 0:HALO, :] = v_scr[:, T:T + HALO, :]

        x = x_ref[...].astype(jnp.float32)
        xn = _ln(x).astype(jnp.bfloat16)
        for part, scr, off in ((0, q_scr, 0), (1, k_scr, HALO), (2, v_scr, HALO)):
            w = pltpu.bitcast(wt_ref[512 * part:512 * part + 512, :], jnp.bfloat16)
            y = jax.lax.dot_general(xn, w, NT, preferred_element_type=jnp.float32)
            if part == 0:
                y = y * scale
            for c in range(8):
                scr[c, off:off + T, :] = y[:, 128 * c:128 * c + 128]

        first = step == 0
        for r in range(0, T, R):
            logits = []
            for w in range(W):
                acc = None
                for c in range(8):
                    t = q_scr[c, r:r + R, :] * k_scr[c, HALO + r - DIL * w:HALO + r - DIL * w + R, :]
                    acc = t if acc is None else acc + t
                if ROT3:
                    acc = (acc + pltpu.roll(acc, 64, 1)) + (pltpu.roll(acc, 32, 1) + pltpu.roll(acc, 96, 1))
                else:
                    acc = acc + pltpu.roll(acc, 64, 1)
                    acc = acc + pltpu.roll(acc, 32, 1)
                if r < DIL * w:
                    row = jax.lax.broadcasted_iota(jnp.int32, (R, 128), 0) + r
                    bad = jnp.logical_and(first, row < DIL * w)
                    acc = jnp.where(bad, -1e9, acc)
                logits.append(acc)
            m = logits[0]
            for l in logits[1:]:
                m = jnp.maximum(m, l)
            p = [jnp.exp(l - m) for l in logits]
            s = p[0]
            for t in p[1:]:
                s = s + t
            inv = 1.0 / s
            p = [t * inv for t in p]
            for c in range(8):
                acc = None
                for w in range(W):
                    t = p[w] * v_scr[c, HALO + r - DIL * w:HALO + r - DIL * w + R, :]
                    acc = t if acc is None else acc + t
                a_scr[r:r + R, 128 * c:128 * c + 128] = acc.astype(jnp.bfloat16)

        wo = pltpu.bitcast(wop_ref[...], jnp.bfloat16)
        h = x + jnp.dot(a_scr[...], wo, preferred_element_type=jnp.float32)
        hn = _ln(h).astype(jnp.bfloat16)
        a = jnp.maximum(jnp.dot(hn, w1_ref[...], preferred_element_type=jnp.float32), 0.0).astype(jnp.bfloat16)
        y = h + jnp.dot(a, w2_ref[...], preferred_element_type=jnp.float32)
        out_ref[...] = y.astype(out_ref.dtype)

    pm = pl.Buffered(1)
    full = lambda a: pl.BlockSpec(a.shape, lambda i: (0, 0), pipeline_mode=pm)
    out = pl.pallas_call(
        kern, grid=(S // T,),
        in_specs=[pl.BlockSpec((T, D), lambda i: (i, 0)), full(A_wqkv), full(A_wo), full(B_w1), full(B_w2)],
        out_specs=pl.BlockSpec((T, D), lambda i: (i, 0)),
        out_shape=jax.ShapeDtypeStruct((S, D), jnp.bfloat16),
        scratch_shapes=[
            pltpu.VMEM((1536, D), jnp.uint32),
            pltpu.VMEM((512, D), jnp.uint32),
            pltpu.VMEM((8, 272, 128), jnp.uint32),
            pltpu.VMEM((8, 272, 128), jnp.uint32),
            pltpu.VMEM((8, T, 128), jnp.float32),
            pltpu.VMEM((8, T + HALO, 128), jnp.float32),
            pltpu.VMEM((8, T + HALO, 128), jnp.float32),
            pltpu.VMEM((T, D), jnp.bfloat16),
        ],
        compiler_params=pltpu.CompilerParams(dimension_semantics=("arbitrary",), vmem_limit_bytes=VMEM_MB << 20),
    )(x2, A_wqkv, A_wo, B_w1, B_w2)
    return out.reshape(1, S, D)
```

```python
import jax
import jax.numpy as jnp
from jax.experimental import pallas as pl
from jax.experimental.pallas import tpu as pltpu

T = 256
LAG = 2
NS = 4
QS, KS = 5, 5
DH, W, DIL = 32, 8, 2
NT = (((1,), (1,)), ((), ()))
ORD = (0, 2, 1, 3, 4, 6, 5, 7, 8, 10, 9, 11, 12, 14, 13, 15)
PITCH = 9


def _ln(x):
    m = jnp.mean(x, axis=-1, keepdims=True)
    c = x - m
    v = jnp.mean(c * c, axis=-1, keepdims=True)
    return c * jax.lax.rsqrt(v + 1e-5)


def _scatter_pairs(src, j, e_ref, o_ref):
    for hl in range(4):
        h = 4 * j + hl
        dst = o_ref if h % 2 else e_ref
        for a in range(8):
            dst[a, pl.ds((h // 2) * 17, 16), :] = src[16 * hl:16 * hl + 16, 128 * a:128 * a + 128]


def _gather_pairs(e_ref, o_ref, dst_ref):
    for dp in range(16):
        for a in range(8):
            ev = e_ref[a, pl.ds(dp, 16, stride=17), :]
            od = o_ref[a, pl.ds(dp, 16, stride=17), :]
            dst_ref[32 * dp:32 * dp + 16, 128 * a:128 * a + 128] = (ev & jnp.uint32(0xFFFF)) | (od << 16)
            dst_ref[32 * dp + 16:32 * dp + 32, 128 * a:128 * a + 128] = (ev >> 16) | (od & jnp.uint32(0xFFFF0000))


def _kernel(x_hbm, wqkv_hbm, wo_hbm, w1_hbm, w2_hbm, out_ref,
            x_buf, wqkv_ref, wo_ref, w1_ref, w2_ref, sems,
            wtq_ref, wtk_ref, wtv_ref, wop_ref, e_ref, o_ref,
            qkv_scr, p_scr, a_scr, xn0_scr, xn1_scr, hn_scr, h_scr, xs_scr, ys_scr):
    S, D = x_hbm.shape
    NB = S // T
    scale = DH ** -0.5
    wt_refs = (wtq_ref, wtk_ref, wtv_ref)
    s = pl.program_id(0)

    def cp_x(b):
        r0 = b * T if isinstance(b, int) else pl.multiple_of(b * T, T)
        return pltpu.make_async_copy(x_hbm.at[pl.ds(r0, T), :], x_buf.at[b % NS], sems.at[7 + b % NS])

    def cp_cols(c0, n, i):
        return pltpu.make_async_copy(wqkv_hbm.at[:, pl.ds(c0, n)], wqkv_ref.at[:, pl.ds(c0, n)], sems.at[i])

    cp_q = lambda i: cp_cols(D // 2 * i, D // 2, i)
    cp_k = lambda: cp_cols(D, D, 2)
    cp_v = lambda: cp_cols(2 * D, D, 3)
    cp_wo = lambda: pltpu.make_async_copy(wo_hbm, wo_ref, sems.at[4])
    cp_w1 = lambda: pltpu.make_async_copy(w1_hbm, w1_ref, sems.at[5])
    cp_w2 = lambda: pltpu.make_async_copy(w2_hbm, w2_ref, sems.at[6])

    def transpose_cols(part, j0, j1):
        for j in range(j0, j1):
            c0 = part * D + 128 * j
            _scatter_pairs(pltpu.bitcast(wqkv_ref[:, c0:c0 + 128].T, jnp.uint32), j, e_ref, o_ref)

    def x_stage(xslot, slot):
        for r in range(16):
            nat = pltpu.bitcast(x_buf[xslot, 16 * r:16 * r + 16, :], jnp.uint32)
            for c in range(8):
                xs_scr[slot, c, pl.ds(PITCH * r, 8), :] = nat[:, 128 * c:128 * c + 128]

    def x_tile(slot, g, mp):
        lo = lambda v: pltpu.bitcast(v << 16, jnp.float32)
        hi = lambda v: pltpu.bitcast(v & jnp.uint32(0xFFFF0000), jnp.float32)
        cols = []
        for c in range(8):
            pa = xs_scr[slot, c, pl.ds(8 * PITCH * g + 2 * mp, 8, stride=PITCH), :]
            pb = xs_scr[slot, c, pl.ds(8 * PITCH * g + 2 * mp + 1, 8, stride=PITCH), :]
            cols.append(jnp.concatenate([lo(pa), lo(pb), hi(pa), hi(pb)], axis=0))
        return jnp.concatenate(cols, axis=1)

    def store_out(y):
        bits = lambda v: pltpu.bitcast(v.astype(jnp.bfloat16).astype(jnp.float32), jnp.uint32)
        for g in range(2):
            pos = {ORD[t]: 128 * g + 8 * t for t in range(16)}
            for c in range(8):
                for m in range(8):
                    lo = bits(y[pos[2 * m]:pos[2 * m] + 8, 128 * c:128 * c + 128])
                    hi = bits(y[pos[2 * m + 1]:pos[2 * m + 1] + 8, 128 * c:128 * c + 128])
                    ys_scr[c, pl.ds(PITCH * (8 * g + m), 8), :] = (lo >> 16) | hi
        for g in range(2):
            for sl in range(8):
                r = 128 * g + 16 * sl
                nat = jnp.concatenate(
                    [ys_scr[c, pl.ds(8 * PITCH * g + sl, 8, stride=PITCH), :] for c in range(8)], axis=1)
                out_ref[r:r + 16, :] = pltpu.bitcast(nat, jnp.bfloat16)

    def ln1(slot, g):
        for mp in range(4):
            y = _ln(x_tile(slot, g, mp)).astype(jnp.bfloat16)
            if g == 0:
                xn0_scr[slot, 32 * mp:32 * mp + 32, :] = y
            else:
                xn1_scr[32 * mp:32 * mp + 32, :] = y

    def ln2(hslot, slot, r0, rows):
        for r in range(r0, r0 + rows, 32):
            hn_scr[slot, r:r + 32, :] = _ln(h_scr[hslot, r:r + 32, :]).astype(jnp.bfloat16)

    def proj(part, slot, groups, chunks=(0, 8)):
        c0, c1 = chunks
        xn = jnp.concatenate([xn0_scr[slot] if g == 0 else xn1_scr[...] for g in groups], axis=0)
        w = pltpu.bitcast(wt_refs[part][64 * c0:64 * c1, :], jnp.bfloat16)
        y = jax.lax.dot_general(xn, w, NT, preferred_element_type=jnp.float32)
        if part == 0:
            y = y * scale
        for gi, g in enumerate(groups):
            for c in range(c0, c1):
                for t in range(16):
                    r = 128 + 8 * ORD[t]
                    qkv_scr[part, c, g, r:r + 8, :] = y[128 * gi + 8 * t:128 * gi + 8 * t + 8,
                                                        128 * (c - c0):128 * (c - c0) + 128]

    def extend(part, g, first):
        sub = jax.lax.broadcasted_iota(jnp.int32, (8, 128), 0)
        for c in range(8):
            for j in range(2, 16):
                cur = qkv_scr[part, c, g, 128 + 8 * j:136 + 8 * j, :]
                if first and g == 0:
                    prev = jnp.broadcast_to(qkv_scr[part, c, 0, 128:129, :], (8, 128))
                else:
                    prev = qkv_scr[part, c, 1 - g, 128 + 8 * j:136 + 8 * j, :]
                qkv_scr[part, c, g, 8 * j:8 * j + 8, :] = pltpu.roll(jnp.where(sub == 7, prev, cur), 1, 0)

    def window(part, c, g, i):
        return [qkv_scr[part, c, g, 128 + 8 * (i - 14 + 2 * n):136 + 8 * (i - 14 + 2 * n), :] for n in range(9)]

    def probs(g, first):
        sub = jax.lax.broadcasted_iota(jnp.int32, (8, 128), 0)
        for t in range(0, 16, 2):
            i = ORD[t]
            logits = [[None] * W, [None] * W]
            for c in range(8):
                ks = window(1, c, g, i)
                for u in range(2):
                    q = qkv_scr[0, c, g, 128 + 8 * (i + 2 * u):136 + 8 * (i + 2 * u), :]
                    for w in range(W):
                        x = q * ks[7 + u - w]
                        logits[u][w] = x if c == 0 else logits[u][w] + x
            for u in range(2):
                lg = []
                for w in range(W):
                    a = logits[u][w]
                    a = (a + pltpu.roll(a, 64, 1)) + (pltpu.roll(a, 32, 1) + pltpu.roll(a, 96, 1))
                    if first and g == 0 and i + 2 * u < DIL * w:
                        a = jnp.where(sub == 0, -1e9, a)
                    lg.append(a)
                m = lg[0]
                for a in lg[1:]:
                    m = jnp.maximum(m, a)
                p = [jnp.exp(a - m) for a in lg]
                tot = p[0]
                for a in p[1:]:
                    tot = tot + a
                inv = 1.0 / tot
                r = 128 * g + 8 * (t + u)
                for w in range(W):
                    p_scr[w, r:r + 8, :] = p[w] * inv

    def weighted_values(g):
        for t in range(0, 16, 2):
            r = 128 * g + 8 * t
            p = [[p_scr[w, r + 8 * u:r + 8 * u + 8, :] for w in range(W)] for u in range(2)]
            for c in range(8):
                vs = window(2, c, g, ORD[t])
                outs = []
                for u in range(2):
                    acc = p[u][0] * vs[7 + u]
                    for w in range(1, W):
                        acc = acc + p[u][w] * vs[7 + u - w]
                    outs.append(acc)
                a_scr[r:r + 16, 128 * c:128 * c + 128] = jnp.concatenate(outs, axis=0).astype(jnp.bfloat16)

    def out_proj(slot, hslot, g):
        wo = pltpu.bitcast(wop_ref[...], jnp.bfloat16)
        att = jnp.dot(a_scr[128 * g:128 * g + 128, :], wo, preferred_element_type=jnp.float32)
        for mp in range(4):
            r = 128 * g + 32 * mp
            h_scr[hslot, r:r + 32, :] = x_tile(slot, g, mp) + att[32 * mp:32 * mp + 32, :]

    @pl.when(s == 0)
    def _():
        for cp in (cp_x(0), cp_q(0), cp_q(1), cp_k(), cp_v(), cp_x(1), cp_wo(), cp_x(2),
                   cp_x(3), cp_w1(), cp_w2()):
            cp.start()
        cp_x(0).wait()
        x_stage(0, 0)
        ln1(0, 0)
        ln1(0, 1)
        for i in range(2):
            cp_q(i).wait()
            transpose_cols(0, 4 * i, 4 * i + 4)
        _gather_pairs(e_ref, o_ref, wtq_ref)
        proj(0, 0, (0, 1), (0, QS))
        cp_k().wait()
        proj(0, 0, (0, 1), (QS, 8))
        transpose_cols(1, 0, 8)
        _gather_pairs(e_ref, o_ref, wtk_ref)
        proj(1, 0, (0, 1), (0, KS))
        cp_v().wait()
        proj(1, 0, (0, 1), (KS, 8))
        extend(1, 0, True)
        extend(1, 1, True)
        transpose_cols(2, 0, 8)
        _gather_pairs(e_ref, o_ref, wtv_ref)
        probs(0, True)
        proj(2, 0, (0,))
        extend(2, 0, True)
        cp_x(1).wait()
        cp_wo().wait()
        probs(1, True)
        proj(2, 0, (1,))
        extend(2, 1, True)
        for j in range(8):
            _scatter_pairs(pltpu.bitcast(wo_ref[128 * j:128 * j + 128, :], jnp.uint32), j, e_ref, o_ref)
        _gather_pairs(e_ref, o_ref, wop_ref)
        x_stage(1, 1)
        ln1(1, 0)
        for g in range(2):
            weighted_values(g)
            out_proj(0, 0, g)
            ln2(0, 0, 128 * g, 128)

    @pl.when(jnp.logical_and(s > 0, s + 1 < NB))
    def _():
        cp_x(s + 1).wait()

    @pl.when(jnp.logical_and(s > 0, s + 3 < NB))
    def _():
        cp_x(s + 3).start()

    @pl.when(jnp.logical_and(s > 0, s < NB))
    def _():
        slot = s % 2
        proj(1, slot, (0,))
        extend(1, 0, False)
        proj(0, slot, (0,))
        proj(2, slot, (0,))
        extend(2, 0, False)
        ln1(slot, 1)
        probs(0, False)
        proj(1, slot, (1,))
        extend(1, 1, False)
        proj(0, slot, (1,))
        weighted_values(0)
        probs(1, False)
        proj(2, slot, (1,))
        extend(2, 1, False)
        x_stage((s + 1) % NS, (s + 1) % 2)
        ln1((s + 1) % 2, 0)
        out_proj(slot, s % NS, 0)
        weighted_values(1)
        out_proj(slot, s % NS, 1)

    @pl.when(s == LAG)
    def _():
        cp_w1().wait()
        cp_w2().wait()

    @pl.when(s >= LAG)
    def _():
        j = s - LAG
        u = jnp.dot(hn_scr[j % 2], w1_ref[...], preferred_element_type=jnp.float32)
        a = jnp.maximum(u, 0.0).astype(jnp.bfloat16)
        store_out(h_scr[j % NS] + jnp.dot(a, w2_ref[...], preferred_element_type=jnp.float32))
        ln2((j + 1) % NS, (j + 1) % 2, 0, T)


@jax.jit
def pallas_sequential_preLN__sliding_local_dilated__dense_activation_relu__prompt_kernel(
    A_x: jax.Array,
    A_wqkv: jax.Array,
    A_wo: jax.Array,
    B_x: jax.Array,
    B_w1: jax.Array,
    B_w2: jax.Array,
):
    _, S, D = A_x.shape
    F = B_w1.shape[1]
    bf16, f32, u32 = jnp.bfloat16, jnp.float32, jnp.uint32
    hbm = pl.BlockSpec(memory_space=pl.ANY)
    out = pl.pallas_call(
        _kernel,
        grid=(S // T + LAG,),
        in_specs=[hbm] * 5,
        out_specs=pl.BlockSpec((T, D), lambda i: (jnp.maximum(i - LAG, 0), 0)),
        out_shape=jax.ShapeDtypeStruct((S, D), bf16),
        scratch_shapes=[
            pltpu.VMEM((NS, T, D), bf16),
            pltpu.VMEM((D, 3 * D), bf16),
            pltpu.VMEM((D, D), bf16),
            pltpu.VMEM((D, F), bf16),
            pltpu.VMEM((F, D), bf16),
            pltpu.SemaphoreType.DMA((7 + NS,)),
            pltpu.VMEM((D // 2, D), u32),
            pltpu.VMEM((D // 2, D), u32),
            pltpu.VMEM((D // 2, D), u32),
            pltpu.VMEM((D // 2, D), u32),
            pltpu.VMEM((8, 272, 128), u32),
            pltpu.VMEM((8, 272, 128), u32),
            pltpu.VMEM((3, 8, 2, 256, 128), f32),
            pltpu.VMEM((W, T, 128), f32),
            pltpu.VMEM((T, D), bf16),
            pltpu.VMEM((2, 128, D), bf16),
            pltpu.VMEM((128, D), bf16),
            pltpu.VMEM((2, T, D), bf16),
            pltpu.VMEM((NS, T, D), f32),
            pltpu.VMEM((2, 8, 16 * PITCH, 128), u32),
            pltpu.VMEM((8, 16 * PITCH, 128), u32),
        ],
        compiler_params=pltpu.CompilerParams(
            dimension_semantics=("arbitrary",),
            vmem_limit_bytes=100 << 20,
            disable_bounds_checks=True,
            flags={"XLA_TPU_EVENLY_DISTRIBUTE_CRITICAL_NODES": True},
        ),
    )(A_x.reshape(S, D), A_wqkv, A_wo, B_w1, B_w2)
    return out.reshape(1, S, D)
```
